```python
import os as _os
_os.environ.setdefault('JAX_PLATFORMS', 'cpu')
import jax
import jax.numpy as jnp

def _softmax(x, axis=-1):
    return jax.nn.softmax(x, axis=axis)

def _gelu(x):
    return jax.nn.gelu(x, approximate=True)

def _silu(x):
    return jax.nn.silu(x)

def _sigmoid(x):
    return jax.nn.sigmoid(x)

def _layernorm(x, axis=-1, eps=1e-05):
    m = jnp.mean(x, axis=axis, keepdims=True)
    v = jnp.var(x, axis=axis, keepdims=True)
    return (x - m) / jnp.sqrt(v + eps)

def _scatter_add(tgt, idx, src, axis=0):
    return tgt.at[idx].add(src)

def _segment_sum(src, seg, n):
    return jax.ops.segment_sum(src, seg, n)

class _Rng:

    def __init__(self, key):
        self._k = key

    def _next(self):
        self._k, sub = jax.random.split(self._k)
        return sub

    def normal(self, shape):
        return jax.random.normal(self._next(), shape, dtype=jnp.bfloat16)

    def randint(self, lo, hi, shape):
        return jax.random.randint(self._next(), shape, lo, hi, dtype=jnp.int32)

    def uniform(self, shape, lo=0.0, hi=1.0):
        return jax.random.uniform(self._next(), shape, jnp.bfloat16, lo, hi)

    def permutation(self, n):
        return jax.random.permutation(self._next(), n)
kernel_name = 'standalone__conformer_family_zipformer__speech'

def setup_inputs():
    _rng = _Rng(jax.random.key(int.from_bytes(__import__("os").urandom(4), "little")))
    _w = lambda a: (lambda t: t.astype(jnp.bfloat16) if jnp.issubdtype(t.dtype, jnp.floating) else t)(jnp.asarray(a))
    B, T, D, K, H = (2, 4000, 144, 3, 4)
    sc = 0.1
    return {'x': _w((lambda *s: _rng.normal(s) * 0.8)(B, T, D)), 'w_ff1a': _w((lambda *s: _rng.normal(s) * 0.8)(D, 4 * D) * sc), 'w_ff1b': _w((lambda *s: _rng.normal(s) * 0.8)(4 * D, D) * sc), 'w_qkv': _w((lambda *s: _rng.normal(s) * 0.8)(D, 3 * D) * sc), 'w_o': _w((lambda *s: _rng.normal(s) * 1.6)(D, D) * sc), 'w_pw1': _w((lambda *s: _rng.normal(s) * 1.6)(D, 2 * D) * sc), 'dw': _w((lambda *s: _rng.normal(s) * 0.4)(K, D)), 'w_pw2': _w((lambda *s: _rng.normal(s) * 0.4)(D, D) * sc), 'w_ff2a': _w((lambda *s: _rng.normal(s) * 0.8)(D, 4 * D) * sc), 'w_ff2b': _w((lambda *s: _rng.normal(s) * 0.8)(4 * D, D) * sc)}

def reference(x, w_ff1a, w_ff1b, w_qkv, w_o, w_pw1, dw, w_pw2, w_ff2a, w_ff2b):
    B, T, D = x.shape
    K = dw.shape[0]
    H = 4
    Dh = D // H
    h = _layernorm(x, axis=-1)
    h = _silu(h @ w_ff1a) @ w_ff1b
    x = x + 0.5 * h
    h = _layernorm(x, axis=-1)
    qkv = h @ w_qkv
    q = (lambda x, *d: x.transpose(*d))(qkv[..., :D].reshape(B, T, H, Dh), 0, 2, 1, 3)
    k = (lambda x, *d: x.transpose(*d))(qkv[..., D:2 * D].reshape(B, T, H, Dh), 0, 2, 1, 3)
    v = (lambda x, *d: x.transpose(*d))(qkv[..., 2 * D:].reshape(B, T, H, Dh), 0, 2, 1, 3)
    scale = Dh ** (-0.5)
    scores = jnp.einsum('bhqd,bhkd->bhqk', q, k) * scale
    p = _softmax(scores, axis=-1)
    att = jnp.einsum('bhqk,bhkd->bhqd', p, v)
    att = (lambda x, *d: x.transpose(*d))(att, 0, 2, 1, 3).reshape(B, T, D)
    x = x + att @ w_o
    h = _layernorm(x, axis=-1)
    h = h @ w_pw1
    a, b = (h[..., :D].copy(), h[..., D:].copy())
    h = a * _sigmoid(b)
    pad = K // 2
    hp = jnp.pad(h, ((0, 0), (pad, pad), (0, 0)))
    c = jnp.zeros_like(h)
    for i in range(K):
        c = c + hp[:, i:i + T, :] * dw[i][None, None, :]
    x = x + _silu(c) @ w_pw2
    h = _layernorm(x, axis=-1)
    h = _silu(h @ w_ff2a) @ w_ff2b
    x = x + 0.5 * h
    return _layernorm(x, axis=-1)
```

```python
import functools
import jax
import jax.numpy as jnp
from jax import lax
import jax.experimental.pallas as pl
import jax.experimental.pallas.tpu as pltpu

F32 = jnp.float32
BF16 = jnp.bfloat16
LOG2E = 1.4426950408889634


def _ln_t(x, eps=1e-5):
    n = x.shape[0]
    m = jnp.sum(x, axis=0, keepdims=True) * (1.0 / n)
    xc = x - m
    v = jnp.sum(xc * xc, axis=0, keepdims=True) * (1.0 / n)
    return xc * lax.rsqrt(v + eps)


def _sigmoid(x):
    return 0.5 * jnp.tanh(0.5 * x) + 0.5


def _silu(x):
    hx = 0.5 * x
    return hx * jnp.tanh(hx) + hx


def _dot(a, b):
    return jnp.dot(a, b, preferred_element_type=F32)


def make_kernel(B, T, D, H, KW, TB, TQ, CK, U, LAG, phases=(1, 2, 3, 4)):
    Dh = D // H
    HP = 48
    TP = -(-T // TB) * TB
    NBLK = TP // TB
    NQ = TP // TQ
    NT = H * NQ
    NBUF = U
    DF = 4 * D
    qscale = (Dh ** -0.5) * LOG2E
    WIN0 = (0, D - 128)
    vstart = [min((h * Dh) // 16 * 16, D - HP) for h in range(H)]
    ones_row = []
    for h in range(H):
        lo, hi = h * Dh - vstart[h], h * Dh - vstart[h] + Dh
        ones_row.append(hi if hi < HP else lo - 1)

    def chunks():
        out = []
        s = 0
        while s < T:
            e = min(s + CK, T)
            out.append((s, e))
            s = e
        return out

    def kernel(x_hbm, w1a, w1bT, wqkv, wo, wpw1, dw, wpw2, w2a, w2bT, o_hbm,
               xbuf, obuf, w1aT, wqkvT, woT, wpw1T, wpw2T, w2aT, dwb,
               xres, qbuf, kbuf, vbuf, attT, gbuf, *rest):
        sb = rest[:NBUF]
        mb = rest[NBUF:2 * NBUF]
        sem_in, sem_out = rest[2 * NBUF:]

        def in_copy(b):
            return pltpu.make_async_copy(x_hbm.at[b], xbuf.at[b], sem_in.at[b])

        def out_copy(b):
            return pltpu.make_async_copy(obuf.at[b], o_hbm.at[b], sem_out.at[b])

        for b in range(B):
            in_copy(b).start()

        w1aT[...] = w1a[...].astype(F32).T.astype(BF16)
        w2aT[...] = w2a[...].astype(F32).T.astype(BF16)
        wpw1T[...] = wpw1[...].astype(F32).T.astype(BF16)
        wpw2T[...] = wpw2[...].astype(F32).T.astype(BF16)
        wqkvT[...] = wqkv[...].astype(F32).T.astype(BF16)
        r = lax.broadcasted_iota(jnp.int32, (D, H * HP), 0)
        c = lax.broadcasted_iota(jnp.int32, (D, H * HP), 1)
        hh = c // HP
        start = jnp.minimum((hh * Dh) // 16 * 16, D - HP)
        feat = start + c % HP
        sel2 = jnp.where((r == feat) & (feat >= hh * Dh) & (feat < (hh + 1) * Dh), 1.0, 0.0).astype(BF16)
        woT[...] = _dot(wo[...].astype(F32).T.astype(BF16), sel2).astype(BF16)
        eye = (lax.broadcasted_iota(jnp.int32, (D, D), 0) == lax.broadcasted_iota(jnp.int32, (D, D), 1)).astype(BF16)
        for k in range(KW):
            dwb[k] = lax.dot_general(eye, jnp.broadcast_to(dw[k:k + 1, :], (128, D)), (((1,), (1,)), ((), ())),
                                     preferred_element_type=F32)
        gbuf[:, 0:128] = jnp.zeros((D, 128), F32)
        gbuf[:, 128 + TP:256 + TP] = jnp.zeros((D, 128), F32)

        def blk(i):
            return pl.ds(pl.multiple_of(i * TB, TB), TB)

        def phase1(b, i):
            xT = xbuf[b, :, blk(i)].astype(F32)
            col = i * TB + lax.broadcasted_iota(jnp.int32, xT.shape, 1)
            xT = jnp.where(col < T, xT, 0.0)
            h = _ln_t(xT).astype(BF16)
            a = _silu(_dot(w1aT[...], h)).astype(BF16)
            x1 = xT + 0.5 * _dot(w1bT[...], a)
            xres[:, blk(i)] = x1
            h = _ln_t(x1).astype(BF16)
            qkv = _dot(wqkvT[...], h)
            for w in range(2):
                qbuf[w, :, blk(i)] = (qkv[WIN0[w]:WIN0[w] + 128] * qscale).astype(BF16)
                kbuf[w, blk(i), :] = qkv[D + WIN0[w]:D + WIN0[w] + 128].T.astype(BF16)
            rr = lax.broadcasted_iota(jnp.int32, (HP, TB), 0)
            for hh in range(H):
                v = qkv[2 * D + vstart[hh]:2 * D + vstart[hh] + HP]
                vbuf[hh, :, blk(i)] = jnp.where(rr == ones_row[hh], 1.0, v).astype(BF16)

        def both(ta, ia, tb, ib):
            if ta is not None:
                ha = ta // NQ
                qa = ta % NQ
                wa = ha // 3
                lo = ha * Dh - wa * WIN0[1]
                qw = qbuf[wa, :, pl.ds(pl.multiple_of(qa * TQ, TQ), TQ)]
                rr = lax.broadcasted_iota(jnp.int32, (128, TQ), 0)
                qT = jnp.where((rr >= lo) & (rr < lo + Dh), qw, jnp.zeros_like(qw))
            if tb is not None:
                hb = tb // NQ
                qb = tb % NQ
                mrow = mb[ib][0:1, :]
            m = None
            acc = None
            for (a, b_) in chunks():
                if tb is not None:
                    p = jnp.exp2(sb[ib][a:b_, :] - mrow).astype(BF16)
                    o = _dot(vbuf[hb, :, a:b_], p)
                    acc = o if acc is None else acc + o
                if ta is not None:
                    s = _dot(kbuf[wa, a:b_, :], qT)
                    sb[ia][a:b_, :] = s
                    mc = jnp.max(s.reshape((b_ - a) // 8, 8, TQ), axis=0)
                    m = mc if m is None else jnp.maximum(m, mc)
            if ta is not None:
                mb[ia][...] = jnp.broadcast_to(jnp.max(m, axis=0, keepdims=True), (8, TQ))
            if tb is not None:
                if isinstance(hb, int):
                    den = acc[ones_row[hb]:ones_row[hb] + 1, :]
                else:
                    orow = jnp.where(hb == 0, ones_row[0], jnp.where(hb == 1, ones_row[1], jnp.where(hb == 2, ones_row[2], ones_row[3])))
                    rr2 = lax.broadcasted_iota(jnp.int32, acc.shape, 0)
                    den = jnp.sum(jnp.where(rr2 == orow, acc, 0.0), axis=0, keepdims=True)
                o = acc * (1.0 / den)
                attT[pl.ds(pl.multiple_of(hb * HP, HP), HP), pl.ds(pl.multiple_of(qb * TQ, TQ), TQ)] = o.astype(BF16)

        def phase2():
            for i in range(LAG):
                both(i, i % NBUF, None, None)
            n_iter = (NT - LAG) // U

            def body(j, _):
                for u in range(U):
                    tb = j * U + u
                    both(tb + LAG, (u + LAG) % NBUF, tb, u % NBUF)
                return 0
            lax.fori_loop(0, n_iter, body, 0)
            for tb in range(n_iter * U, NT):
                ta = tb + LAG
                both(ta if ta < NT else None, ta % NBUF, tb, tb % NBUF)

        def phase3(i):
            x2 = xres[:, blk(i)] + _dot(woT[...], attT[:, blk(i)])
            xres[:, blk(i)] = x2
            h = _ln_t(x2).astype(BF16)
            u = _dot(wpw1T[...], h)
            g = u[:D] * _sigmoid(u[D:])
            col = i * TB + lax.broadcasted_iota(jnp.int32, g.shape, 1)
            g = jnp.where(col < T, g, 0.0)
            gbuf[:, pl.ds(pl.multiple_of(128 + i * TB, 128), TB)] = g

        def phase4(b, i):
            gw = gbuf[:, pl.ds(pl.multiple_of(i * TB, TB), TB + 256)]
            gc = gw[:, 128:128 + TB]
            gl = pltpu.roll(gw, 1, 1)[:, 128:128 + TB]
            gr = pltpu.roll(gw, TB + 255, 1)[:, 128:128 + TB]
            rep = TB // 128
            d0 = jnp.concatenate([dwb[0]] * rep, axis=1)
            d1 = jnp.concatenate([dwb[1]] * rep, axis=1)
            d2 = jnp.concatenate([dwb[2]] * rep, axis=1)
            c = gl * d0 + gc * d1 + gr * d2
            x3 = xres[:, blk(i)] + _dot(wpw2T[...], _silu(c).astype(BF16))
            h = _ln_t(x3).astype(BF16)
            a = _silu(_dot(w2aT[...], h)).astype(BF16)
            x4 = x3 + 0.5 * _dot(w2bT[...], a)
            y = _ln_t(x4)
            obuf[b, :, blk(i)] = y.astype(BF16)

        def batch(b, _):
            in_copy(b).wait()
            if 1 in phases:
                lax.fori_loop(0, NBLK, lambda i, c: (phase1(b, i), 0)[1], 0)
            if 2 in phases:
                phase2()
            if 3 in phases:
                lax.fori_loop(0, NBLK, lambda i, c: (phase3(i), 0)[1], 0)
            if 4 in phases:
                lax.fori_loop(0, NBLK, lambda i, c: (phase4(b, i), 0)[1], 0)
            out_copy(b).start()
            return 0

        lax.fori_loop(0, B, batch, 0)
        for b in range(B):
            out_copy(b).wait()

    scratch = [
        pltpu.VMEM((B, D, T), BF16),
        pltpu.VMEM((B, D, T), BF16),
        pltpu.VMEM((DF, D), BF16),
        pltpu.VMEM((3 * D, D), BF16),
        pltpu.VMEM((D, H * HP), BF16),
        pltpu.VMEM((2 * D, D), BF16),
        pltpu.VMEM((D, D), BF16),
        pltpu.VMEM((DF, D), BF16),
        pltpu.VMEM((KW, D, 128), F32),
        pltpu.VMEM((D, TP), F32),
        pltpu.VMEM((2, 128, TP), BF16),
        pltpu.VMEM((2, TP, 128), BF16),
        pltpu.VMEM((H, HP, TP), BF16),
        pltpu.VMEM((H * HP, TP), BF16),
        pltpu.VMEM((D, TP + 256), F32),
    ] + [pltpu.VMEM((T, TQ), F32)] * NBUF + [pltpu.VMEM((8, TQ), F32)] * NBUF + [
        pltpu.SemaphoreType.DMA((B,)), pltpu.SemaphoreType.DMA((B,))]
    return kernel, scratch


@jax.jit
def pallas_standalone__conformer_family_zipformer__speech_kernel(
    x: jax.Array,
    w_ff1a: jax.Array,
    w_ff1b: jax.Array,
    w_qkv: jax.Array,
    w_o: jax.Array,
    w_pw1: jax.Array,
    dw: jax.Array,
    w_pw2: jax.Array,
    w_ff2a: jax.Array,
    w_ff2b: jax.Array,
):
    B, T, D = x.shape
    kernel, scratch = make_kernel(B, T, D, 4, dw.shape[0], 512, 256, 256, 4, 2)
    vm = pl.BlockSpec(memory_space=pltpu.VMEM)
    oT = pl.pallas_call(
        kernel,
        out_shape=jax.ShapeDtypeStruct((B, D, T), x.dtype),
        in_specs=[pl.BlockSpec(memory_space=pl.ANY)] + [vm] * 9,
        out_specs=pl.BlockSpec(memory_space=pl.ANY),
        scratch_shapes=scratch,
        compiler_params=pltpu.CompilerParams(vmem_limit_bytes=110 * 1024 * 1024),
        name="zipformer",
    )(jnp.transpose(x, (0, 2, 1)), w_ff1a, w_ff1b.T, w_qkv, w_o, w_pw1, dw, w_pw2, w_ff2a, w_ff2b.T)
    return jnp.transpose(oT, (0, 2, 1))
```

```python
import contextlib
import jax
import jax.numpy as jnp
from jax import lax
import jax.experimental.pallas as pl
import jax.experimental.pallas.tpu as pltpu

F32 = jnp.float32
BF16 = jnp.bfloat16
U32 = jnp.uint32
LOG2E = 1.4426950408889634
LANES = 128


def _ln_t(x, eps=1e-5):
    n = x.shape[0]
    m = jnp.sum(x, axis=0, keepdims=True) * (1.0 / n)
    xc = x - m
    v = jnp.sum(xc * xc, axis=0, keepdims=True) * (1.0 / n)
    return xc * lax.rsqrt(v + eps)


def _sigmoid(x):
    return 0.5 * jnp.tanh(0.5 * x) + 0.5


def _silu(x):
    hx = 0.5 * x
    return hx * jnp.tanh(hx) + hx


def _dot(a, b):
    return jnp.dot(a, b, preferred_element_type=F32)


def _tr(w):
    return w.astype(F32).T.astype(BF16)


def make_kernel(B, T, D, H, KW, TB1, TB3, TB4, SB4, TQ, CK, U, LAG, NBUF, scopes=False):
    Dh = D // H
    HP = 48
    TP = -(-T // 2048) * 2048
    DF = 4 * D
    qscale = (Dh ** -0.5) * LOG2E
    WIN0 = (0, D - LANES)
    win_of = [0 if (h + 1) * Dh <= LANES else 1 for h in range(H)]
    vstart = [min((h * Dh) // 16 * 16, D - HP) for h in range(H)]
    ones_row = []
    for h in range(H):
        lo, hi = h * Dh - vstart[h], h * Dh - vstart[h] + Dh
        ones_row.append(hi if hi < HP else lo - 1)
    assert U % NBUF == 0 and LAG < NBUF and U % H == 0

    NFULL = T // TQ
    rest = T - NFULL * TQ
    NHALF = rest // LANES
    REM = rest - NHALF * LANES
    assert REM * H <= LANES
    steps = [("t", h, j * TQ, TQ) for j in range(NFULL) for h in range(H)]
    steps += [("t", h, NFULL * TQ + j * LANES, LANES) for j in range(NHALF) for h in range(H)]
    REM0 = NFULL * TQ + NHALF * LANES
    if REM:
        steps.append(("r", None, REM0, LANES))
    NS = len(steps)

    def scope(name):
        return jax.named_scope(name) if scopes else contextlib.nullcontext()

    def chunks():
        out = []
        s = 0
        while s < T:
            e = min(s + CK, T)
            out.append((s, e))
            s = e
        return out

    XCH = 2048
    NXC = TP // XCH

    def kernel(x_hbm, w1a_h, w1bT_h, wqkv_h, wo_h, wpw1_h, dw_h, wpw2_h, w2a_h, w2bT_h, o_hbm,
               xbuf, obuf, w1a, w1bT, wqkv, wo, wpw1, dw, wpw2, w2a, w2bT,
               w1aT, wqkvT, woT, wpw1T, wpw2T, w2aT, dwb,
               xres, qbuf, kbuf, vbuf, attT, gbuf, *rest_refs):
        sb = rest_refs[:NBUF]
        mb = rest_refs[NBUF:2 * NBUF]
        sem_x, sem_w, sem_out = rest_refs[2 * NBUF:]
        NB4 = TP // TB4

        def x_copy(b, i):
            w = min(XCH, T - i * XCH)
            return pltpu.make_async_copy(x_hbm.at[b, :, pl.ds(i * XCH, w)], xbuf.at[b, :, pl.ds(i * XCH, w)],
                                         sem_x.at[b * NXC + i])

        def out_copy(b, i):
            w = min(TB4, T - i * TB4)
            return pltpu.make_async_copy(obuf.at[b, :, pl.ds(i * TB4, w)], o_hbm.at[b, :, pl.ds(i * TB4, w)],
                                         sem_out.at[b * NB4 + i])

        w_pairs = [(w1a_h, w1a), (w1bT_h, w1bT), (wqkv_h, wqkv), (wo_h, wo), (wpw1_h, wpw1), (dw_h, dw),
                   (wpw2_h, wpw2), (w2a_h, w2a), (w2bT_h, w2bT)]
        w_copy = [pltpu.make_async_copy(s, d, sem_w.at[i]) for i, (s, d) in enumerate(w_pairs)]

        w_copy[0].start()
        x_copy(0, 0).start()
        w_copy[2].start()
        w_copy[1].start()

        def start_rest():
            for i in range(1, NXC):
                x_copy(0, i).start()
            for i in range(3, 9):
                w_copy[i].start()
            for b in range(1, B):
                for i in range(NXC):
                    x_copy(b, i).start()

        with scope("prep"):
            gbuf[:, 0:LANES] = jnp.zeros((D // 2, LANES), U32)
            gbuf[:, LANES + TP:2 * LANES + TP] = jnp.zeros((D // 2, LANES), U32)
            w_copy[0].wait()
            w1aT[...] = _tr(w1a[...])
            w_copy[2].wait()
            wqkvT[...] = _tr(wqkv[...])
            w_copy[1].wait()

        def prep2():
            for i in range(3, 9):
                w_copy[i].wait()
            w2aT[...] = _tr(w2a[...])
            wpw1T[...] = _tr(wpw1[...])
            wpw2T[...] = _tr(wpw2[...])
            r = lax.broadcasted_iota(jnp.int32, (D, H * HP), 0)
            c = lax.broadcasted_iota(jnp.int32, (D, H * HP), 1)
            hh = c // HP
            start = jnp.minimum((hh * Dh) // 16 * 16, D - HP)
            feat = start + c % HP
            sel = jnp.where((r == feat) & (feat >= hh * Dh) & (feat < (hh + 1) * Dh), 1.0, 0.0).astype(BF16)
            woT[...] = _dot(_tr(wo[...]), sel).astype(BF16)
            eye = (lax.broadcasted_iota(jnp.int32, (D, D), 0)
                   == lax.broadcasted_iota(jnp.int32, (D, D), 1)).astype(BF16)
            for k in range(KW):
                dwb[k] = lax.dot_general(eye, jnp.broadcast_to(dw[k:k + 1, :], (LANES, D)),
                                         (((1,), (1,)), ((), ())), preferred_element_type=F32)

        def cols(c0, w):
            if isinstance(c0, int):
                return pl.ds(c0, w)
            return pl.ds(pl.multiple_of(c0, LANES), w)

        def phase1(b, c0, w):
            cs = cols(c0, w)
            xT = xbuf[b, :, cs].astype(F32)
            col = c0 + lax.broadcasted_iota(jnp.int32, xT.shape, 1)
            xT = jnp.where(col < T, xT, 0.0)
            h = _ln_t(xT).astype(BF16)
            a = _silu(_dot(w1aT[...], h)).astype(BF16)
            x1 = xT + 0.5 * _dot(w1bT[...], a)
            xres[:, cs] = x1
            h = _ln_t(x1).astype(BF16)
            qkv = _dot(wqkvT[...], h)
            for wi in range(2):
                qbuf[wi, :, cs] = (qkv[WIN0[wi]:WIN0[wi] + LANES] * qscale).astype(BF16)
                kk = qkv[D + WIN0[wi]:D + WIN0[wi] + LANES].T.astype(BF16)
                kbuf[wi, pl.ds(pl.multiple_of(c0 // 2, w // 2), w // 2), :] = pltpu.bitcast(kk, U32)
            rr = lax.broadcasted_iota(jnp.int32, (HP, w), 0)
            for hh in range(H):
                v = qkv[2 * D + vstart[hh]:2 * D + vstart[hh] + HP]
                vbuf[hh, :, cs] = pltpu.bitcast(jnp.where(rr == ones_row[hh], 1.0, v).astype(BF16), U32)

        def head_rows(h):
            lo = h * Dh - WIN0[win_of[h]]
            return lo, lo + Dh

        def both(sa, ia, sbs, ib):
            if sa is not None:
                kind_a, ha, qa, wa = sa
                rr = lax.broadcasted_iota(jnp.int32, (LANES, wa), 0)
                if kind_a == "t":
                    lo, hi = head_rows(ha)
                    qw = qbuf[win_of[ha], :, cols(qa, wa)]
                    qTs = [(win_of[ha], jnp.where((rr >= lo) & (rr < hi), qw, jnp.zeros_like(qw)))]
                else:
                    lane = lax.broadcasted_iota(jnp.int32, (LANES, wa), 1)
                    qTs = []
                    for wi in range(2):
                        q = qbuf[wi, :, cols(qa, wa)].astype(F32)
                        q = jnp.where(lane < REM, q, 0.0)
                        acc_q = jnp.zeros_like(q)
                        for h in range(H):
                            if win_of[h] != wi:
                                continue
                            lo, hi = head_rows(h)
                            qh = q if h == 0 else pltpu.roll(q, h * REM, 1)
                            acc_q = jnp.where((rr >= lo) & (rr < hi) & (lane >= h * REM) & (lane < (h + 1) * REM),
                                              qh, acc_q)
                        qTs.append((wi, acc_q.astype(BF16)))
            if sbs is not None:
                kind_b, hb, qb, wb = sbs
                mrow = mb[ib][0:1, 0:wb]
            m = None
            acc = None
            for (a, b_) in chunks():
                if sbs is not None:
                    p = jnp.exp2(sb[ib][a:b_, 0:wb] - mrow).astype(BF16)
                    if kind_b == "t":
                        vv = pltpu.bitcast(vbuf[hb, :, a:b_], BF16)
                    else:
                        vv = pltpu.bitcast(vbuf[:, :, a:b_].reshape(H * HP // 2, b_ - a), BF16)
                    o = _dot(vv, p)
                    acc = o if acc is None else acc + o
                if sa is not None:
                    s = None
                    for (wi, qT) in qTs:
                        sw = _dot(pltpu.bitcast(kbuf[wi, a // 2:b_ // 2, :], BF16), qT)
                        s = sw if s is None else s + sw
                    sb[ia][a:b_, 0:wa] = s
                    mc = jnp.max(s.reshape((b_ - a) // 8, 8, wa), axis=0)
                    m = mc if m is None else jnp.maximum(m, mc)
            if sa is not None:
                mb[ia][:, 0:wa] = jnp.broadcast_to(jnp.max(m, axis=0, keepdims=True), (8, wa))
            if sbs is not None:
                if kind_b == "t":
                    den = acc[ones_row[hb]:ones_row[hb] + 1, :]
                    o = acc * (1.0 / den)
                    attT[hb * HP:(hb + 1) * HP, cols(qb, wb)] = o.astype(BF16)
                else:
                    for h in range(H):
                        ah = acc[h * HP:(h + 1) * HP]
                        den = ah[ones_row[h]:ones_row[h] + 1, :]
                        o = ah * (1.0 / den)
                        if h:
                            o = pltpu.roll(o, LANES - h * REM, 1)
                        attT[h * HP:(h + 1) * HP, cols(qb, wb)] = o.astype(BF16)

        def phase2():
            with scope("ph2pro"):
                for i in range(LAG):
                    both(steps[i], i % NBUF, None, None)
            n_iter = (NFULL * H - LAG) // U

            def body(j, _):
                q0 = j * (U // H) * TQ
                for u in range(U):
                    ua = u + LAG
                    both(("t", ua % H, q0 + (ua // H) * TQ, TQ), ua % NBUF,
                         ("t", u % H, q0 + (u // H) * TQ, TQ), u % NBUF)
                return 0
            with scope("ph2main"):
                lax.fori_loop(0, n_iter, body, 0)
            for tb in range(n_iter * U, NS):
                ta = tb + LAG
                both(steps[ta] if ta < NS else None, ta % NBUF, steps[tb], tb % NBUF)

        def phase3(c0, w):
            cs = cols(c0, w)
            x2 = xres[:, cs] + _dot(woT[...], attT[:, cs])
            xres[:, cs] = x2
            h = _ln_t(x2).astype(BF16)
            u = _dot(wpw1T[...], h)
            g = u[:D] * _sigmoid(u[D:])
            col = c0 + lax.broadcasted_iota(jnp.int32, g.shape, 1)
            g = jnp.where(col < T, g, 0.0)
            gbuf[:, cols(LANES + c0, w)] = pltpu.bitcast(g.astype(BF16), U32)

        def p4_a(c0, w):
            gw = gbuf[:, cols(c0, w + 2 * LANES)]
            gc = pltpu.bitcast(gw[:, LANES:LANES + w], BF16).astype(F32)
            gl = pltpu.bitcast(pltpu.roll(gw, 1, 1)[:, LANES:LANES + w], BF16).astype(F32)
            gr = pltpu.bitcast(pltpu.roll(gw, w + 2 * LANES - 1, 1)[:, LANES:LANES + w], BF16).astype(F32)
            rep = w // LANES
            d0 = jnp.concatenate([dwb[0]] * rep, axis=1)
            d1 = jnp.concatenate([dwb[1]] * rep, axis=1)
            d2 = jnp.concatenate([dwb[2]] * rep, axis=1)
            c = gl * d0 + gc * d1 + gr * d2
            return _silu(c).astype(BF16)

        def p4_b(c0, w, sc):
            x3 = xres[:, cols(c0, w)] + _dot(wpw2T[...], sc)
            return x3, _ln_t(x3).astype(BF16)

        def p4_c(x3, h):
            a = _silu(_dot(w2aT[...], h)).astype(BF16)
            return x3 + 0.5 * _dot(w2bT[...], a)

        def p4_d(b, c0, w, x4):
            obuf[b, :, cols(c0, w)] = _ln_t(x4).astype(BF16)

        def phase4_block(b, base):
            n = TB4 // SB4
            w = SB4
            st_b = {}
            st_c = {}
            for s in range(n + 2):
                if s < n:
                    sc = p4_a(base + s * w, w)
                    st_b[s] = p4_b(base + s * w, w, sc)
                if 0 <= s - 1 < n:
                    st_c[s - 1] = p4_c(*st_b[s - 1])
                if 0 <= s - 2 < n:
                    p4_d(b, base + (s - 2) * w, w, st_c[s - 2])

        def batch(b, _):
            def body1(i, _):
                for ci in range(1, NXC):
                    @pl.when((b == 0) & (i * TB1 == ci * XCH))
                    def _():
                        x_copy(0, ci).wait()
                phase1(b, i * TB1, TB1)
                return 0
            with scope("inwait"):
                for bb in range(B):
                    @pl.when(b == bb)
                    def _():
                        for i in range(NXC):
                            if i == 0 or bb > 0:
                                x_copy(bb, i).wait()
                        if bb == 0:
                            start_rest()
            with scope("ph1"):
                lax.fori_loop(0, TP // TB1, body1, 0)
            with scope("prep2"):
                @pl.when(b == 0)
                def _():
                    prep2()
            with scope("ph2"):
                phase2()
            with scope("ph3"):
                lax.fori_loop(0, TP // TB3, lambda i, c: (phase3(i * TB3, TB3), 0)[1], 0)

            def body4(t, _):
                phase4_block(b, t * TB4)
                for i in range(NB4):
                    @pl.when(t == i)
                    def _():
                        out_copy(b, i).start()
                return 0
            with scope("ph4"):
                lax.fori_loop(0, NB4, body4, 0)
            return 0

        lax.fori_loop(0, B, batch, 0)
        with scope("outwait"):
            for b in range(B):
                for i in range(NB4):
                    out_copy(b, i).wait()

    NB4_ = TP // TB4
    scratch = [
        pltpu.VMEM((B, D, T), BF16),
        pltpu.VMEM((B, D, T), BF16),
        pltpu.VMEM((D, DF), BF16),
        pltpu.VMEM((D, DF), BF16),
        pltpu.VMEM((D, 3 * D), BF16),
        pltpu.VMEM((D, D), BF16),
        pltpu.VMEM((D, 2 * D), BF16),
        pltpu.VMEM((KW, D), BF16),
        pltpu.VMEM((D, D), BF16),
        pltpu.VMEM((D, DF), BF16),
        pltpu.VMEM((D, DF), BF16),
        pltpu.VMEM((DF, D), BF16),
        pltpu.VMEM((3 * D, D), BF16),
        pltpu.VMEM((D, H * HP), BF16),
        pltpu.VMEM((2 * D, D), BF16),
        pltpu.VMEM((D, D), BF16),
        pltpu.VMEM((DF, D), BF16),
        pltpu.VMEM((KW, D, LANES), F32),
        pltpu.VMEM((D, TP), F32),
        pltpu.VMEM((2, LANES, TP), BF16),
        pltpu.VMEM((2, TP // 2, LANES), U32),
        pltpu.VMEM((H, HP // 2, TP), U32),
        pltpu.VMEM((H * HP, TP), BF16),
        pltpu.VMEM((D // 2, TP + 2 * LANES), U32),
    ] + [pltpu.VMEM((T, TQ), F32)] * NBUF + [pltpu.VMEM((8, TQ), F32)] * NBUF + [
        pltpu.SemaphoreType.DMA((B * NXC,)), pltpu.SemaphoreType.DMA((9,)), pltpu.SemaphoreType.DMA((B * NB4_,))]
    return kernel, scratch


@jax.jit
def pallas_standalone__conformer_family_zipformer__speech_kernel(
    x: jax.Array,
    w_ff1a: jax.Array,
    w_ff1b: jax.Array,
    w_qkv: jax.Array,
    w_o: jax.Array,
    w_pw1: jax.Array,
    dw: jax.Array,
    w_pw2: jax.Array,
    w_ff2a: jax.Array,
    w_ff2b: jax.Array,
):
    B, T, D = x.shape
    kernel, scratch = make_kernel(B, T, D, 4, dw.shape[0], TB1=2048, TB3=2048, TB4=2048, SB4=512, TQ=256, CK=256, U=8, LAG=2, NBUF=4)
    hbm = pl.BlockSpec(memory_space=pl.ANY)
    oT = pl.pallas_call(
        kernel,
        out_shape=jax.ShapeDtypeStruct((B, D, T), x.dtype),
        in_specs=[hbm] * 10,
        out_specs=hbm,
        scratch_shapes=scratch,
        compiler_params=pltpu.CompilerParams(vmem_limit_bytes=120 * 1024 * 1024),
        name="zipformer",
    )(jnp.transpose(x, (0, 2, 1)), w_ff1a, w_ff1b.T, w_qkv, w_o, w_pw1, dw, w_pw2, w_ff2a, w_ff2b.T)
    return jnp.transpose(oT, (0, 2, 1))
```

```python
import contextlib
import jax
import jax.numpy as jnp
from jax import lax
import jax.experimental.pallas as pl
import jax.experimental.pallas.tpu as pltpu

F32 = jnp.float32
BF16 = jnp.bfloat16
U32 = jnp.uint32
LOG2E = 1.4426950408889634
LANES = 128


def _ln_t(x, eps=1e-5):
    n = x.shape[0]
    m = jnp.sum(x, axis=0, keepdims=True) * (1.0 / n)
    xc = x - m
    v = jnp.sum(xc * xc, axis=0, keepdims=True) * (1.0 / n)
    return xc * lax.rsqrt(v + eps)


def _sigmoid(x):
    return 0.5 * jnp.tanh(0.5 * x) + 0.5


def _silu(x):
    hx = 0.5 * x
    return hx * jnp.tanh(hx) + hx


def _dot(a, b):
    return jnp.dot(a, b, preferred_element_type=F32)


def _tr(w):
    return w.astype(F32).T.astype(BF16)


def make_kernel(B, T, D, H, KW, TB1, SB1, TB3, TB4, SB4, TQ, CK, U, LAG, NBUF, scopes=False, INLINE_OUT=True):
    Dh = D // H
    HP = 48
    TP = -(-T // 2048) * 2048
    DF = 4 * D
    qscale = (Dh ** -0.5) * LOG2E
    WIN0 = (0, D - LANES)
    win_of = [0 if (h + 1) * Dh <= LANES else 1 for h in range(H)]
    vstart = [min((h * Dh) // 16 * 16, D - HP) for h in range(H)]
    ones_row = []
    for h in range(H):
        lo, hi = h * Dh - vstart[h], h * Dh - vstart[h] + Dh
        ones_row.append(hi if hi < HP else lo - 1)
    assert U % NBUF == 0 and LAG < NBUF and U % H == 0

    NFULL = T // TQ
    rest = T - NFULL * TQ
    NHALF = rest // LANES
    REM = rest - NHALF * LANES
    assert REM * H <= LANES
    steps = [("t", h, j * TQ, TQ) for j in range(NFULL) for h in range(H)]
    steps += [("t", h, NFULL * TQ + j * LANES, LANES) for j in range(NHALF) for h in range(H)]
    REM0 = NFULL * TQ + NHALF * LANES
    if REM:
        steps.append(("r", None, REM0, LANES))
    NS = len(steps)

    def scope(name):
        return jax.named_scope(name) if scopes else contextlib.nullcontext()

    def chunks():
        out = []
        s = 0
        while s < T:
            e = min(s + CK, T)
            out.append((s, e))
            s = e
        return out

    XCH = 2048
    NXC = TP // XCH

    def kernel(x_hbm, w1a_h, w1bT_h, wqkv_h, wo_h, wpw1_h, dw_h, wpw2_h, w2a_h, w2bT_h, o_hbm,
               xbuf, obuf, w1a, w1bT, wqkv, wo, wpw1, dw, wpw2, w2a, w2bT,
               w1aT, wqkvT, woT, wpw1T, wpw2T, w2aT, dwb,
               xres, qbuf, kbuf, vbuf, attT, gbuf, *rest_refs):
        sb = rest_refs[:NBUF]
        mb = rest_refs[NBUF:2 * NBUF]
        sem_x, sem_w, sem_out = rest_refs[2 * NBUF:]
        NB4 = TP // SB4
        NSB = TB4 // SB4

        def cols(c0, w):
            if isinstance(c0, int):
                return pl.ds(c0, w)
            return pl.ds(pl.multiple_of(c0, LANES), w)

        def x_copy(b, i):
            w = min(XCH, T - i * XCH)
            return pltpu.make_async_copy(x_hbm.at[b, :, pl.ds(i * XCH, w)], xbuf.at[b, :, pl.ds(i * XCH, w)],
                                         sem_x.at[b * NXC + i])

        def out_copy(b, i, c0=None):
            if c0 is None:
                c0 = i * SB4
                w = min(SB4, T - c0)
            else:
                w = SB4
            return pltpu.make_async_copy(obuf.at[b, :, cols(c0, w)], o_hbm.at[b, :, cols(c0, w)],
                                         sem_out.at[b * NB4 + i])

        w_pairs = [(w1a_h, w1a), (w1bT_h, w1bT), (wqkv_h, wqkv), (wo_h, wo), (wpw1_h, wpw1), (dw_h, dw),
                   (wpw2_h, wpw2), (w2a_h, w2a), (w2bT_h, w2bT)]
        w_copy = [pltpu.make_async_copy(s, d, sem_w.at[i]) for i, (s, d) in enumerate(w_pairs)]

        w_copy[0].start()
        x_copy(0, 0).start()
        w_copy[2].start()
        w_copy[1].start()

        def start_rest():
            for i in range(1, NXC):
                x_copy(0, i).start()
            for i in range(3, 9):
                w_copy[i].start()
            for b in range(1, B):
                for i in range(NXC):
                    x_copy(b, i).start()

        with scope("prep"):
            gbuf[:, 0:LANES] = jnp.zeros((D // 2, LANES), U32)
            gbuf[:, LANES + TP:2 * LANES + TP] = jnp.zeros((D // 2, LANES), U32)
            w_copy[0].wait()
            w1aT[...] = _tr(w1a[...])
            w_copy[2].wait()
            wqkvT[...] = _tr(wqkv[...])
            w_copy[1].wait()

        def prep2():
            w2aT[...] = _tr(w2a[...])
            wpw1T[...] = _tr(wpw1[...])
            wpw2T[...] = _tr(wpw2[...])
            r = lax.broadcasted_iota(jnp.int32, (D, H * HP), 0)
            c = lax.broadcasted_iota(jnp.int32, (D, H * HP), 1)
            hh = c // HP
            start = jnp.minimum((hh * Dh) // 16 * 16, D - HP)
            feat = start + c % HP
            sel = jnp.where((r == feat) & (feat >= hh * Dh) & (feat < (hh + 1) * Dh), 1.0, 0.0).astype(BF16)
            woT[...] = _dot(_tr(wo[...]), sel).astype(BF16)
            eye = (lax.broadcasted_iota(jnp.int32, (D, D), 0)
                   == lax.broadcasted_iota(jnp.int32, (D, D), 1)).astype(BF16)
            for k in range(KW):
                dwb[k] = lax.dot_general(eye, jnp.broadcast_to(dw[k:k + 1, :], (LANES, D)),
                                         (((1,), (1,)), ((), ())), preferred_element_type=F32)

        def p1_a(b, c0, w):
            cs = cols(c0, w)
            xT = xbuf[b, :, cs].astype(F32)
            col = c0 + lax.broadcasted_iota(jnp.int32, xT.shape, 1)
            xT = jnp.where(col < T, xT, 0.0)
            h = _ln_t(xT).astype(BF16)
            a = _silu(_dot(w1aT[...], h)).astype(BF16)
            x1 = xT + 0.5 * _dot(w1bT[...], a)
            xres[:, cs] = x1
            return _ln_t(x1).astype(BF16)

        def p1_b(c0, w, h):
            cs = cols(c0, w)
            qkv = _dot(wqkvT[...], h)
            for wi in range(2):
                qbuf[wi, :, cs] = (qkv[WIN0[wi]:WIN0[wi] + LANES] * qscale).astype(BF16)
                kk = qkv[D + WIN0[wi]:D + WIN0[wi] + LANES].T.astype(BF16)
                kbuf[wi, pl.ds(pl.multiple_of(c0 // 2, w // 2), w // 2), :] = pltpu.bitcast(kk, U32)
            rr = lax.broadcasted_iota(jnp.int32, (HP, w), 0)
            for hh in range(H):
                v = qkv[2 * D + vstart[hh]:2 * D + vstart[hh] + HP]
                vbuf[hh, :, cs] = pltpu.bitcast(jnp.where(rr == ones_row[hh], 1.0, v).astype(BF16), U32)

        def phase1(b, c0, w):
            n = w // SB1
            hs = {}
            for s in range(n + 1):
                if s < n:
                    hs[s] = p1_a(b, c0 + s * SB1, SB1)
                if s >= 1:
                    p1_b(c0 + (s - 1) * SB1, SB1, hs.pop(s - 1))

        def head_rows(h):
            lo = h * Dh - WIN0[win_of[h]]
            return lo, lo + Dh

        def both(sa, ia, sbs, ib):
            if sa is not None:
                kind_a, ha, qa, wa = sa
                rr = lax.broadcasted_iota(jnp.int32, (LANES, wa), 0)
                if kind_a == "t":
                    lo, hi = head_rows(ha)
                    qw = qbuf[win_of[ha], :, cols(qa, wa)]
                    qTs = [(win_of[ha], jnp.where((rr >= lo) & (rr < hi), qw, jnp.zeros_like(qw)))]
                else:
                    lane = lax.broadcasted_iota(jnp.int32, (LANES, wa), 1)
                    qTs = []
                    for wi in range(2):
                        q = qbuf[wi, :, cols(qa, wa)].astype(F32)
                        q = jnp.where(lane < REM, q, 0.0)
                        acc_q = jnp.zeros_like(q)
                        for h in range(H):
                            if win_of[h] != wi:
                                continue
                            lo, hi = head_rows(h)
                            qh = q if h == 0 else pltpu.roll(q, h * REM, 1)
                            acc_q = jnp.where((rr >= lo) & (rr < hi) & (lane >= h * REM) & (lane < (h + 1) * REM),
                                              qh, acc_q)
                        qTs.append((wi, acc_q.astype(BF16)))
            if sbs is not None:
                kind_b, hb, qb, wb = sbs
                mrow = mb[ib][0:1, 0:wb]
            m = None
            acc = None
            for (a, b_) in chunks():
                if sbs is not None:
                    p = jnp.exp2(sb[ib][a:b_, 0:wb] - mrow).astype(BF16)
                    if kind_b == "t":
                        vv = pltpu.bitcast(vbuf[hb, :, a:b_], BF16)
                    else:
                        vv = pltpu.bitcast(vbuf[:, :, a:b_].reshape(H * HP // 2, b_ - a), BF16)
                    o = _dot(vv, p)
                    acc = o if acc is None else acc + o
                if sa is not None:
                    s = None
                    for (wi, qT) in qTs:
                        sw = _dot(pltpu.bitcast(kbuf[wi, a // 2:b_ // 2, :], BF16), qT)
                        s = sw if s is None else s + sw
                    sb[ia][a:b_, 0:wa] = s
                    mc = jnp.max(s.reshape((b_ - a) // 8, 8, wa), axis=0)
                    m = mc if m is None else jnp.maximum(m, mc)
            if sa is not None:
                mb[ia][:, 0:wa] = jnp.broadcast_to(jnp.max(m, axis=0, keepdims=True), (8, wa))
            if sbs is not None:
                if kind_b == "t":
                    den = acc[ones_row[hb]:ones_row[hb] + 1, :]
                    o = acc * (1.0 / den)
                    attT[hb * HP:(hb + 1) * HP, cols(qb, wb)] = o.astype(BF16)
                else:
                    for h in range(H):
                        ah = acc[h * HP:(h + 1) * HP]
                        den = ah[ones_row[h]:ones_row[h] + 1, :]
                        o = ah * (1.0 / den)
                        if h:
                            o = pltpu.roll(o, LANES - h * REM, 1)
                        attT[h * HP:(h + 1) * HP, cols(qb, wb)] = o.astype(BF16)

        def phase2():
            with scope("ph2pro"):
                for i in range(LAG):
                    both(steps[i], i % NBUF, None, None)
            n_iter = (NFULL * H - LAG) // U

            def body(j, _):
                q0 = j * (U // H) * TQ
                for u in range(U):
                    ua = u + LAG
                    both(("t", ua % H, q0 + (ua // H) * TQ, TQ), ua % NBUF,
                         ("t", u % H, q0 + (u // H) * TQ, TQ), u % NBUF)
                return 0
            with scope("ph2main"):
                lax.fori_loop(0, n_iter, body, 0)
            for tb in range(n_iter * U, NS):
                ta = tb + LAG
                both(steps[ta] if ta < NS else None, ta % NBUF, steps[tb], tb % NBUF)

        def phase3(c0, w):
            cs = cols(c0, w)
            x2 = xres[:, cs] + _dot(woT[...], attT[:, cs])
            xres[:, cs] = x2
            h = _ln_t(x2).astype(BF16)
            u = _dot(wpw1T[...], h)
            g = u[:D] * _sigmoid(u[D:])
            col = c0 + lax.broadcasted_iota(jnp.int32, g.shape, 1)
            g = jnp.where(col < T, g, 0.0)
            gbuf[:, cols(LANES + c0, w)] = pltpu.bitcast(g.astype(BF16), U32)

        def p4_a(c0, w):
            gw = gbuf[:, cols(c0, w + 2 * LANES)]
            gc = pltpu.bitcast(gw[:, LANES:LANES + w], BF16).astype(F32)
            gl = pltpu.bitcast(pltpu.roll(gw, 1, 1)[:, LANES:LANES + w], BF16).astype(F32)
            gr = pltpu.bitcast(pltpu.roll(gw, w + 2 * LANES - 1, 1)[:, LANES:LANES + w], BF16).astype(F32)
            rep = w // LANES
            d0 = jnp.concatenate([dwb[0]] * rep, axis=1)
            d1 = jnp.concatenate([dwb[1]] * rep, axis=1)
            d2 = jnp.concatenate([dwb[2]] * rep, axis=1)
            c = gl * d0 + gc * d1 + gr * d2
            return _silu(c).astype(BF16)

        def p4_b(c0, w, sc):
            x3 = xres[:, cols(c0, w)] + _dot(wpw2T[...], sc)
            return x3, _ln_t(x3).astype(BF16)

        def p4_c(x3, h):
            a = _silu(_dot(w2aT[...], h)).astype(BF16)
            return x3 + 0.5 * _dot(w2bT[...], a)

        def p4_d(b, c0, w, x4):
            obuf[b, :, cols(c0, w)] = _ln_t(x4).astype(BF16)

        def phase4_block(b, t):
            base = t * TB4
            n = NSB
            w = SB4
            st_b = {}
            st_c = {}
            for s in range(n + 2):
                if s < n:
                    sc = p4_a(base + s * w, w)
                    st_b[s] = p4_b(base + s * w, w, sc)
                if 0 <= s - 1 < n:
                    st_c[s - 1] = p4_c(*st_b.pop(s - 1))
                if 0 <= s - 2 < n:
                    p4_d(b, base + (s - 2) * w, w, st_c.pop(s - 2))
                    if s - 2 < n - 1 and INLINE_OUT:
                        out_copy(b, t * n + s - 2, base + (s - 2) * w).start()

        def batch(b, _):
            def body1(i, _):
                for ci in range(1, NXC):
                    @pl.when((b == 0) & (i * TB1 == ci * XCH))
                    def _():
                        x_copy(0, ci).wait()
                phase1(b, i * TB1, TB1)
                return 0
            with scope("inwait"):
                for bb in range(B):
                    @pl.when(b == bb)
                    def _():
                        for i in range(NXC):
                            if i == 0 or bb > 0:
                                x_copy(bb, i).wait()
                        if bb == 0:
                            start_rest()
            with scope("ph1"):
                lax.fori_loop(0, TP // TB1, body1, 0)
            with scope("prep2"):
                @pl.when(b == 0)
                def _():
                    for i in range(3, 9):
                        w_copy[i].wait()
                    prep2()
            with scope("ph2"):
                phase2()
            with scope("ph3"):
                lax.fori_loop(0, TP // TB3, lambda i, c: (phase3(i * TB3, TB3), 0)[1], 0)

            def body4(t, _):
                phase4_block(b, t)
                for i in range(TP // TB4):
                    @pl.when(t == i)
                    def _():
                        for s in range(NSB):
                            if s == NSB - 1 or not INLINE_OUT:
                                out_copy(b, i * NSB + s).start()
                return 0
            with scope("ph4"):
                lax.fori_loop(0, TP // TB4, body4, 0)
            return 0

        lax.fori_loop(0, B, batch, 0)
        with scope("outwait"):
            for b in range(B):
                for i in range(NB4):
                    out_copy(b, i).wait()

    NB4_ = TP // SB4
    scratch = [
        pltpu.VMEM((B, D, T), BF16),
        pltpu.VMEM((B, D, T), BF16),
        pltpu.VMEM((D, DF), BF16),
        pltpu.VMEM((D, DF), BF16),
        pltpu.VMEM((D, 3 * D), BF16),
        pltpu.VMEM((D, D), BF16),
        pltpu.VMEM((D, 2 * D), BF16),
        pltpu.VMEM((KW, D), BF16),
        pltpu.VMEM((D, D), BF16),
        pltpu.VMEM((D, DF), BF16),
        pltpu.VMEM((D, DF), BF16),
        pltpu.VMEM((DF, D), BF16),
        pltpu.VMEM((3 * D, D), BF16),
        pltpu.VMEM((D, H * HP), BF16),
        pltpu.VMEM((2 * D, D), BF16),
        pltpu.VMEM((D, D), BF16),
        pltpu.VMEM((DF, D), BF16),
        pltpu.VMEM((KW, D, LANES), F32),
        pltpu.VMEM((D, TP), F32),
        pltpu.VMEM((2, LANES, TP), BF16),
        pltpu.VMEM((2, TP // 2, LANES), U32),
        pltpu.VMEM((H, HP // 2, TP), U32),
        pltpu.VMEM((H * HP, TP), BF16),
        pltpu.VMEM((D // 2, TP + 2 * LANES), U32),
    ] + [pltpu.VMEM((T, TQ), F32)] * NBUF + [pltpu.VMEM((8, TQ), F32)] * NBUF + [
        pltpu.SemaphoreType.DMA((B * NXC,)), pltpu.SemaphoreType.DMA((9,)), pltpu.SemaphoreType.DMA((B * NB4_,))]
    return kernel, scratch


@jax.jit
def pallas_standalone__conformer_family_zipformer__speech_kernel(
    x: jax.Array,
    w_ff1a: jax.Array,
    w_ff1b: jax.Array,
    w_qkv: jax.Array,
    w_o: jax.Array,
    w_pw1: jax.Array,
    dw: jax.Array,
    w_pw2: jax.Array,
    w_ff2a: jax.Array,
    w_ff2b: jax.Array,
):
    B, T, D = x.shape
    kernel, scratch = make_kernel(B, T, D, 4, dw.shape[0], TB1=2048, SB1=512, TB3=2048, TB4=2048, SB4=512, TQ=128, CK=256, U=20, LAG=2, NBUF=4)
    hbm = pl.BlockSpec(memory_space=pl.ANY)
    oT = pl.pallas_call(
        kernel,
        out_shape=jax.ShapeDtypeStruct((B, D, T), x.dtype),
        in_specs=[hbm] * 10,
        out_specs=hbm,
        scratch_shapes=scratch,
        compiler_params=pltpu.CompilerParams(vmem_limit_bytes=120 * 1024 * 1024),
        name="zipformer",
    )(jnp.transpose(x, (0, 2, 1)), w_ff1a, w_ff1b.T, w_qkv, w_o, w_pw1, dw, w_pw2, w_ff2a, w_ff2b.T)
    return jnp.transpose(oT, (0, 2, 1))
```

```python
import jax
import jax.numpy as jnp
from jax import lax
import jax.experimental.pallas as pl
import jax.experimental.pallas.tpu as pltpu

F32 = jnp.float32
BF16 = jnp.bfloat16
U32 = jnp.uint32
LOG2E = 1.4426950408889634
LANES = 128


def _ln_t(x, eps=1e-5):
    n = x.shape[0]
    m = jnp.sum(x, axis=0, keepdims=True) * (1.0 / n)
    xc = x - m
    v = jnp.sum(xc * xc, axis=0, keepdims=True) * (1.0 / n)
    return xc * lax.rsqrt(v + eps)


def _sigmoid(x):
    return 0.5 * jnp.tanh(0.5 * x) + 0.5


def _silu(x):
    hx = 0.5 * x
    return hx * jnp.tanh(hx) + hx


def _dot(a, b):
    return jnp.dot(a, b, preferred_element_type=F32)


def _tr(w):
    return w.astype(F32).T.astype(BF16)


def _make_kernel(B, T, D, H, KW):
    TB = 2048
    SB = 512
    TQ = LANES
    CK = 256
    U = 20
    LAG = 2
    NBUF = 4

    Dh = D // H
    HP = 48
    TP = -(-T // TB) * TB
    DF = 4 * D
    NBLK = TP // TB
    NSB = TB // SB
    NOUT = TP // SB
    qscale = (Dh ** -0.5) * LOG2E
    assert LANES < D <= 2 * LANES and D % 16 == 0 and U % NBUF == 0 and LAG < NBUF and U % H == 0
    WIN0 = (0, D - LANES)
    win_of = [0 if (h + 1) * Dh <= LANES else 1 for h in range(H)]
    assert all(h * Dh >= WIN0[win_of[h]] for h in range(H))
    vstart = [min((h * Dh) // 16 * 16, D - HP) for h in range(H)]
    ones_row = []
    for h in range(H):
        lo, hi = h * Dh - vstart[h], h * Dh - vstart[h] + Dh
        assert 0 <= lo and hi <= HP and Dh < HP
        ones_row.append(hi if hi < HP else lo - 1)

    NFULL = T // TQ
    REM = T - NFULL * TQ
    assert REM * H <= LANES
    steps = [("t", h, j * TQ) for j in range(NFULL) for h in range(H)]
    if REM:
        steps.append(("r", None, NFULL * TQ))
    NS = len(steps)
    key_chunks = [(s, min(s + CK, T)) for s in range(0, T, CK)]

    def kernel(x_hbm, w1a_h, w1bT_h, wqkv_h, wo_h, wpw1_h, dw_h, wpw2_h, w2a_h, w2bT_h, o_hbm,
               xbuf, obuf, w1a, w1bT, wqkv, wo, wpw1, dw, wpw2, w2a, w2bT,
               w1aT, wqkvT, woT, wpw1T, wpw2T, w2aT, dwb,
               xres, qbuf, kbuf, vbuf, attT, gbuf, *rest_refs):
        sb = rest_refs[:NBUF]
        mb = rest_refs[NBUF:2 * NBUF]
        sem_x, sem_w, sem_out = rest_refs[2 * NBUF:]

        def cols(c0, w):
            if isinstance(c0, int):
                return pl.ds(c0, w)
            return pl.ds(pl.multiple_of(c0, LANES), w)

        def x_copy(b, i):
            w = min(TB, T - i * TB)
            return pltpu.make_async_copy(x_hbm.at[b, :, pl.ds(i * TB, w)], xbuf.at[b, :, pl.ds(i * TB, w)],
                                         sem_x.at[b * NBLK + i])

        def out_copy(b, i, c0=None):
            if c0 is None:
                c0 = i * SB
                w = min(SB, T - c0)
            else:
                w = SB
            return pltpu.make_async_copy(obuf.at[b, :, cols(c0, w)], o_hbm.at[b, :, cols(c0, w)],
                                         sem_out.at[b * NOUT + i])

        w_pairs = [(w1a_h, w1a), (w1bT_h, w1bT), (wqkv_h, wqkv), (wo_h, wo), (wpw1_h, wpw1), (dw_h, dw),
                   (wpw2_h, wpw2), (w2a_h, w2a), (w2bT_h, w2bT)]
        w_copy = [pltpu.make_async_copy(s, d, sem_w.at[i]) for i, (s, d) in enumerate(w_pairs)]
        N_EARLY = 3

        for i in range(N_EARLY):
            w_copy[i].start()
        x_copy(0, 0).start()

        def start_rest():
            for i in range(1, NBLK):
                x_copy(0, i).start()
            for i in range(N_EARLY, len(w_copy)):
                w_copy[i].start()
            for b in range(1, B):
                for i in range(NBLK):
                    x_copy(b, i).start()

        for k in range(KW):
            gbuf[k, :, 0:LANES] = jnp.zeros((D // 2, LANES), U32)
            gbuf[k, :, LANES + TP:2 * LANES + TP] = jnp.zeros((D // 2, LANES), U32)
        w_copy[0].wait()
        w1aT[...] = _tr(w1a[...])
        w_copy[2].wait()
        wqkvT[...] = _tr(wqkv[...])
        w_copy[1].wait()

        def prep_late():
            for i in range(N_EARLY, len(w_copy)):
                w_copy[i].wait()
            w2aT[...] = _tr(w2a[...])
            wpw1T[...] = _tr(wpw1[...])
            wpw2T[...] = _tr(wpw2[...])
            r = lax.broadcasted_iota(jnp.int32, (D, H * HP), 0)
            c = lax.broadcasted_iota(jnp.int32, (D, H * HP), 1)
            hh = c // HP
            feat = jnp.minimum((hh * Dh) // 16 * 16, D - HP) + c % HP
            sel = jnp.where((r == feat) & (feat >= hh * Dh) & (feat < (hh + 1) * Dh), 1.0, 0.0).astype(BF16)
            woT[...] = _dot(_tr(wo[...]), sel).astype(BF16)
            eye = (lax.broadcasted_iota(jnp.int32, (D, D), 0)
                   == lax.broadcasted_iota(jnp.int32, (D, D), 1)).astype(BF16)
            for k in range(KW):
                dwb[k] = lax.dot_general(eye, jnp.broadcast_to(dw[k:k + 1, :], (LANES, D)),
                                         (((1,), (1,)), ((), ())), preferred_element_type=F32)

        def p1_a(b, c0, w):
            cs = cols(c0, w)
            xT = xbuf[b, :, cs].astype(F32)
            col = c0 + lax.broadcasted_iota(jnp.int32, xT.shape, 1)
            xT = jnp.where(col < T, xT, 0.0)
            h = _ln_t(xT).astype(BF16)
            a = _silu(_dot(w1aT[...], h)).astype(BF16)
            x1 = xT + 0.5 * _dot(w1bT[...], a)
            xres[:, cs] = x1
            return _ln_t(x1).astype(BF16)

        def p1_b(c0, w, h):
            cs = cols(c0, w)
            qkv = _dot(wqkvT[...], h)
            for wi in range(2):
                qbuf[wi, :, cs] = (qkv[WIN0[wi]:WIN0[wi] + LANES] * qscale).astype(BF16)
                kk = qkv[D + WIN0[wi]:D + WIN0[wi] + LANES].T.astype(BF16)
                kbuf[wi, pl.ds(pl.multiple_of(c0 // 2, w // 2), w // 2), :] = pltpu.bitcast(kk, U32)
            rr = lax.broadcasted_iota(jnp.int32, (HP, w), 0)
            for hh in range(H):
                v = qkv[2 * D + vstart[hh]:2 * D + vstart[hh] + HP]
                vbuf[hh, :, cs] = pltpu.bitcast(jnp.where(rr == ones_row[hh], 1.0, v).astype(BF16), U32)

        def phase1(b, base):
            hs = {}
            for s in range(NSB + 1):
                if s < NSB:
                    hs[s] = p1_a(b, base + s * SB, SB)
                if s >= 1:
                    p1_b(base + (s - 1) * SB, SB, hs.pop(s - 1))

        def head_rows(h):
            lo = h * Dh - WIN0[win_of[h]]
            return lo, lo + Dh

        def both(sa, ia, sbs, ib):
            if sa is not None:
                kind_a, ha, qa = sa
                rr = lax.broadcasted_iota(jnp.int32, (LANES, TQ), 0)
                if kind_a == "t":
                    lo, hi = head_rows(ha)
                    qw = qbuf[win_of[ha], :, cols(qa, TQ)]
                    qTs = [(win_of[ha], jnp.where((rr >= lo) & (rr < hi), qw, jnp.zeros_like(qw)))]
                else:
                    lane = lax.broadcasted_iota(jnp.int32, (LANES, TQ), 1)
                    qTs = []
                    for wi in range(2):
                        q = qbuf[wi, :, cols(qa, TQ)].astype(F32)
                        qm = jnp.zeros_like(q)
                        for h in range(H):
                            if win_of[h] != wi:
                                continue
                            lo, hi = head_rows(h)
                            qh = q if h == 0 else pltpu.roll(q, h * REM, 1)
                            qm = jnp.where((rr >= lo) & (rr < hi) & (lane >= h * REM) & (lane < (h + 1) * REM),
                                           qh, qm)
                        qTs.append((wi, qm.astype(BF16)))
            if sbs is not None:
                kind_b, hb, qb = sbs
                mrow = mb[ib][0:1, :]
            m = None
            acc = None
            for (a, e) in key_chunks:
                if sbs is not None:
                    p = jnp.exp2(sb[ib][a:e, :] - mrow).astype(BF16)
                    if kind_b == "t":
                        vv = pltpu.bitcast(vbuf[hb, :, a:e], BF16)
                    else:
                        vv = pltpu.bitcast(vbuf[:, :, a:e].reshape(H * HP // 2, e - a), BF16)
                    o = _dot(vv, p)
                    acc = o if acc is None else acc + o
                if sa is not None:
                    s = None
                    for (wi, qT) in qTs:
                        sw = _dot(pltpu.bitcast(kbuf[wi, a // 2:e // 2, :], BF16), qT)
                        s = sw if s is None else s + sw
                    sb[ia][a:e, :] = s
                    mc = jnp.max(s.reshape((e - a) // 8, 8, TQ), axis=0)
                    m = mc if m is None else jnp.maximum(m, mc)
            if sa is not None:
                mb[ia][...] = jnp.broadcast_to(jnp.max(m, axis=0, keepdims=True), (8, TQ))
            if sbs is not None:
                for h in ([hb] if kind_b == "t" else range(H)):
                    ah = acc if kind_b == "t" else acc[h * HP:(h + 1) * HP]
                    o = ah * (1.0 / ah[ones_row[h]:ones_row[h] + 1, :])
                    if kind_b == "r" and h:
                        o = pltpu.roll(o, LANES - h * REM, 1)
                    attT[h * HP:(h + 1) * HP, cols(qb, TQ)] = o.astype(BF16)

        def phase2():
            for i in range(LAG):
                both(steps[i], i % NBUF, None, None)
            n_iter = (NFULL * H - LAG) // U

            def body(j, carry):
                q0 = j * (U // H) * TQ
                for u in range(U):
                    ua = u + LAG
                    both(("t", ua % H, q0 + (ua // H) * TQ), ua % NBUF,
                         ("t", u % H, q0 + (u // H) * TQ), u % NBUF)
                return carry
            lax.fori_loop(0, n_iter, body, 0)
            for tb in range(n_iter * U, NS):
                ta = tb + LAG
                both(steps[ta] if ta < NS else None, ta % NBUF, steps[tb], tb % NBUF)

        def phase3(c0, w):
            cs = cols(c0, w)
            x2 = xres[:, cs] + _dot(woT[...], attT[:, cs])
            xres[:, cs] = x2
            h = _ln_t(x2).astype(BF16)
            u = _dot(wpw1T[...], h)
            g = u[:D] * _sigmoid(u[D:])
            col = c0 + lax.broadcasted_iota(jnp.int32, g.shape, 1)
            g = jnp.where(col < T, g, 0.0)
            for k in range(KW):
                dk = jnp.concatenate([dwb[k]] * (w // LANES), axis=1)
                gbuf[k, :, cols(LANES + c0, w)] = pltpu.bitcast((g * dk).astype(BF16), U32)

        def p4_a(c0, w):
            wn = cols(c0, w + 2 * LANES)
            c = None
            for k in range(KW):
                sh = KW // 2 - k
                assert abs(sh) < LANES
                if sh == 0:
                    gk = gbuf[k, :, cols(LANES + c0, w)]
                else:
                    gk = pltpu.roll(gbuf[k, :, wn], sh % (w + 2 * LANES), 1)[:, LANES:LANES + w]
                gk = pltpu.bitcast(gk, BF16).astype(F32)
                c = gk if c is None else c + gk
            return _silu(c).astype(BF16)

        def p4_b(c0, w, sc):
            x3 = xres[:, cols(c0, w)] + _dot(wpw2T[...], sc)
            return x3, _ln_t(x3).astype(BF16)

        def p4_c(x3, h):
            a = _silu(_dot(w2aT[...], h)).astype(BF16)
            return x3 + 0.5 * _dot(w2bT[...], a)

        def phase4(b, t):
            base = t * TB
            st_b = {}
            st_c = {}
            for s in range(NSB + 2):
                if s < NSB:
                    st_b[s] = p4_b(base + s * SB, SB, p4_a(base + s * SB, SB))
                if 0 <= s - 1 < NSB:
                    st_c[s - 1] = p4_c(*st_b.pop(s - 1))
                if 0 <= s - 2 < NSB:
                    c0 = base + (s - 2) * SB
                    obuf[b, :, cols(c0, SB)] = _ln_t(st_c.pop(s - 2)).astype(BF16)
                    if s - 2 < NSB - 1:
                        out_copy(b, t * NSB + s - 2, c0).start()

        def batch(b, carry):
            for bb in range(B):
                @pl.when(b == bb)
                def _():
                    for i in range(NBLK):
                        if i == 0 or bb > 0:
                            x_copy(bb, i).wait()
                    if bb == 0:
                        start_rest()

            def body1(i, c):
                for ci in range(1, NBLK):
                    @pl.when((b == 0) & (i == ci))
                    def _():
                        x_copy(0, ci).wait()
                phase1(b, i * TB)
                return c
            lax.fori_loop(0, NBLK, body1, 0)

            @pl.when(b == 0)
            def _():
                prep_late()

            phase2()

            def body3(i, c):
                phase3(i * TB, TB)
                return c
            lax.fori_loop(0, NBLK, body3, 0)

            def body4(t, c):
                phase4(b, t)
                for i in range(NBLK):
                    @pl.when(t == i)
                    def _():
                        out_copy(b, i * NSB + NSB - 1).start()
                return c
            lax.fori_loop(0, NBLK, body4, 0)
            return carry

        lax.fori_loop(0, B, batch, 0)
        for b in range(B):
            for i in range(NOUT):
                out_copy(b, i).wait()

    scratch = [
        pltpu.VMEM((B, D, T), BF16),
        pltpu.VMEM((B, D, T), BF16),
        pltpu.VMEM((D, DF), BF16),
        pltpu.VMEM((D, DF), BF16),
        pltpu.VMEM((D, 3 * D), BF16),
        pltpu.VMEM((D, D), BF16),
        pltpu.VMEM((D, 2 * D), BF16),
        pltpu.VMEM((KW, D), BF16),
        pltpu.VMEM((D, D), BF16),
        pltpu.VMEM((D, DF), BF16),
        pltpu.VMEM((D, DF), BF16),
        pltpu.VMEM((DF, D), BF16),
        pltpu.VMEM((3 * D, D), BF16),
        pltpu.VMEM((D, H * HP), BF16),
        pltpu.VMEM((2 * D, D), BF16),
        pltpu.VMEM((D, D), BF16),
        pltpu.VMEM((DF, D), BF16),
        pltpu.VMEM((KW, D, LANES), F32),
        pltpu.VMEM((D, TP), F32),
        pltpu.VMEM((2, LANES, TP), BF16),
        pltpu.VMEM((2, TP // 2, LANES), U32),
        pltpu.VMEM((H, HP // 2, TP), U32),
        pltpu.VMEM((H * HP, TP), BF16),
        pltpu.VMEM((KW, D // 2, TP + 2 * LANES), U32),
    ] + [pltpu.VMEM((T, TQ), F32)] * NBUF + [pltpu.VMEM((8, TQ), F32)] * NBUF + [
        pltpu.SemaphoreType.DMA((B * NBLK,)),
        pltpu.SemaphoreType.DMA((9,)),
        pltpu.SemaphoreType.DMA((B * NOUT,)),
    ]
    return kernel, scratch


@jax.jit
def pallas_standalone__conformer_family_zipformer__speech_kernel(
    x: jax.Array,
    w_ff1a: jax.Array,
    w_ff1b: jax.Array,
    w_qkv: jax.Array,
    w_o: jax.Array,
    w_pw1: jax.Array,
    dw: jax.Array,
    w_pw2: jax.Array,
    w_ff2a: jax.Array,
    w_ff2b: jax.Array,
):
    B, T, D = x.shape
    kernel, scratch = _make_kernel(B, T, D, 4, dw.shape[0])
    hbm = pl.BlockSpec(memory_space=pl.ANY)
    oT = pl.pallas_call(
        kernel,
        out_shape=jax.ShapeDtypeStruct((B, D, T), x.dtype),
        in_specs=[hbm] * 10,
        out_specs=hbm,
        scratch_shapes=scratch,
        compiler_params=pltpu.CompilerParams(vmem_limit_bytes=100 * 1024 * 1024),
        name="zipformer",
    )(jnp.transpose(x, (0, 2, 1)), w_ff1a, w_ff1b.T, w_qkv, w_o, w_pw1, dw, w_pw2, w_ff2a, w_ff2b.T)
    return jnp.transpose(oT, (0, 2, 1))
```
